```python
import os as _os
_os.environ.setdefault("JAX_PLATFORMS", "cpu")
import jax
import jax.numpy as jnp

def _softmax(x, axis=-1):
    return jax.nn.softmax(x, axis=axis)
def _gelu(x):
    return jax.nn.gelu(x, approximate=True)
def _silu(x):
    return jax.nn.silu(x)
def _sigmoid(x):
    return jax.nn.sigmoid(x)
def _layernorm(x, axis=-1, eps=1e-5):
    m = jnp.mean(x, axis=axis, keepdims=True)
    v = jnp.var(x, axis=axis, keepdims=True)
    return (x - m) / jnp.sqrt(v + eps)
def _scatter_add(tgt, idx, src, axis=0):
    return tgt.at[idx].add(src)
def _segment_sum(src, seg, n):
    return jax.ops.segment_sum(src, seg, n)
class _Rng:
    def __init__(self, key):
        self._k = key
    def _next(self):
        self._k, sub = jax.random.split(self._k)
        return sub
    def normal(self, shape):
        return jax.random.normal(self._next(), shape, dtype=jnp.bfloat16)
    def randint(self, lo, hi, shape):
        return jax.random.randint(self._next(), shape, lo, hi, dtype=jnp.int32)
    def uniform(self, shape, lo=0.0, hi=1.0):
        return jax.random.uniform(self._next(), shape, jnp.bfloat16, lo, hi)
    def permutation(self, n):
        return jax.random.permutation(self._next(), n)


kernel_name = 'standalone__gqa_softmax__near_ridge'

def setup_inputs():
    _rng = _Rng(jax.random.key(int.from_bytes(__import__("os").urandom(4), "little")))
    _w = (lambda a: (lambda t: t.astype(jnp.bfloat16) if jnp.issubdtype(t.dtype, jnp.floating) else t)(jnp.asarray(a)))
    B, Hq, Hkv, Sq, Sk, D = 8, 16, 8, 160, 2048, 256
    return {
        "q": _w((lambda *s: _rng.normal(s) * 0.05)(B, Hq, Sq, D)),
        "k": _w((lambda *s: _rng.normal(s) * 3.2)(B, Hkv, Sk, D)),
        "v": _w((lambda *s: _rng.normal(s) * 0.05)(B, Hkv, Sk, D)),
    }

def reference(q, k, v):
    B, Hq, Sq, D = q.shape
    Hkv = k.shape[1]
    rep = Hq // Hkv
    k = jnp.repeat(k, rep, axis=1)
    v = jnp.repeat(v, rep, axis=1)
    scale = D ** -0.5
    scores = jnp.einsum("bhqd,bhkd->bhqk", q, k) * scale
    p = _softmax(scores, axis=-1)
    return jnp.einsum("bhqk,bhkd->bhqd", p, v)
```

```python
import jax
import jax.numpy as jnp
import jax.experimental.pallas as pl
import jax.experimental.pallas.tpu as pltpu


@jax.jit
def pallas_standalone__gqa_softmax__near_ridge_kernel(
    q: jax.Array,
    k: jax.Array,
    v: jax.Array,
):
    B, Hq, Sq, D = q.shape
    Hkv, Sk = k.shape[1], k.shape[2]
    rep = Hq // Hkv
    M = rep * Sq
    G = B * Hkv
    hpb = 2
    qr = q.reshape(G, M, D)
    kr = k.reshape(G, Sk, D)
    vr = v.reshape(G, Sk, D)
    scale = D ** -0.5

    def kernel(q_ref, k_ref, v_ref, o_ref):
        for h in range(hpb):
            qq = q_ref[h] * jnp.asarray(scale, q_ref.dtype)
            s = jax.lax.dot_general(qq, k_ref[h], (((1,), (1,)), ((), ())),
                                    preferred_element_type=jnp.float32)
            m = jnp.max(s, axis=-1, keepdims=True)
            p = jnp.exp(s - m)
            l = jnp.sum(p, axis=-1, keepdims=True)
            o = jnp.dot(p.astype(jnp.bfloat16), v_ref[h],
                        preferred_element_type=jnp.float32)
            o_ref[h] = (o / l).astype(o_ref.dtype)

    out = pl.pallas_call(
        kernel,
        grid=(G // hpb,),
        in_specs=[
            pl.BlockSpec((hpb, M, D), lambda i: (i, 0, 0)),
            pl.BlockSpec((hpb, Sk, D), lambda i: (i, 0, 0)),
            pl.BlockSpec((hpb, Sk, D), lambda i: (i, 0, 0)),
        ],
        out_specs=pl.BlockSpec((hpb, M, D), lambda i: (i, 0, 0)),
        out_shape=jax.ShapeDtypeStruct((G, M, D), q.dtype),
        compiler_params=pltpu.CompilerParams(
            dimension_semantics=("parallel",),
            vmem_limit_bytes=96 * 1024 * 1024),
    )(qr, kr, vr)
    return out.reshape(B, Hq, Sq, D)
```

```python
import math

import jax
import jax.numpy as jnp
from jax import lax
import jax.experimental.pallas as pl
import jax.experimental.pallas.tpu as pltpu

_NT = (((1,), (1,)), ((), ()))


@jax.jit
def pallas_standalone__gqa_softmax__near_ridge_kernel(
    q: jax.Array,
    k: jax.Array,
    v: jax.Array,
):
    B, Hq, Sq, D = q.shape
    Hkv, Sk = k.shape[1], k.shape[2]
    rep = Hq // Hkv
    M = rep * Sq
    G = B * Hkv
    hpb = 2
    CS = 512
    NC = Sk // CS
    qr = q.reshape(G, M, D)
    kr = k.reshape(G, Sk, D)
    vr = v.reshape(G, Sk, D)
    c_exp = (D ** -0.5) * math.log2(math.e)
    items = [(h, j) for h in range(hpb) for j in range(NC)]

    def kernel(q_ref, k_ref, v_ref, o_ref):
        def qk(it):
            h, j = it
            return lax.dot_general(q_ref[h], k_ref[h, j * CS:(j + 1) * CS, :], _NT,
                                   preferred_element_type=jnp.float32)

        s_next = qk(items[0])
        m = l = acc = None
        for n, (h, j) in enumerate(items):
            s = s_next
            if n + 1 < len(items):
                s_next = qk(items[n + 1])
            mc = jnp.max(s, axis=-1, keepdims=True)
            m_new = mc if j == 0 else jnp.maximum(m, mc)
            p = jnp.exp2((s - m_new) * c_exp).astype(jnp.bfloat16)
            pv = jnp.dot(p, v_ref[h, j * CS:(j + 1) * CS, :],
                         preferred_element_type=jnp.float32)
            ls = jnp.sum(p.astype(jnp.float32), axis=-1, keepdims=True)
            if j == 0:
                l = ls
                acc = pv
            else:
                alpha = jnp.exp2((m - m_new) * c_exp)
                l = l * alpha + ls
                acc = acc * alpha + pv
            m = m_new
            if j == NC - 1:
                o_ref[h] = (acc * pl.reciprocal(l, approx=False)).astype(o_ref.dtype)

    out = pl.pallas_call(
        kernel,
        grid=(G // hpb,),
        in_specs=[
            pl.BlockSpec((hpb, M, D), lambda i: (i, 0, 0)),
            pl.BlockSpec((hpb, Sk, D), lambda i: (i, 0, 0)),
            pl.BlockSpec((hpb, Sk, D), lambda i: (i, 0, 0)),
        ],
        out_specs=pl.BlockSpec((hpb, M, D), lambda i: (i, 0, 0)),
        out_shape=jax.ShapeDtypeStruct((G, M, D), q.dtype),
        compiler_params=pltpu.CompilerParams(
            dimension_semantics=("parallel",),
            vmem_limit_bytes=100 * 1024 * 1024),
    )(qr, kr, vr)
    return out.reshape(B, Hq, Sq, D)
```

```python
import math

import jax
import jax.numpy as jnp
from jax import lax
import jax.experimental.pallas as pl
import jax.experimental.pallas.tpu as pltpu

_NT = (((1,), (1,)), ((), ()))


@jax.jit
def pallas_standalone__gqa_softmax__near_ridge_kernel(
    q: jax.Array,
    k: jax.Array,
    v: jax.Array,
):
    B, Hq, Sq, D = q.shape
    Hkv, Sk = k.shape[1], k.shape[2]
    rep = Hq // Hkv
    M = rep * Sq
    G = B * Hkv
    hpb = 2
    CS = 256
    AHEAD = 2
    NC = Sk // CS
    qr = q.reshape(G, M, D)
    kr = k.reshape(G, Sk, D)
    vr = v.reshape(G, Sk, D)
    c_exp = (D ** -0.5) * math.log2(math.e)
    items = [(h, j) for j in range(NC) for h in range(hpb)]

    def kernel(q_ref, k_ref, v_ref, o_ref):
        def qk(it):
            h, j = it
            return lax.dot_general(q_ref[h], k_ref[h, j * CS:(j + 1) * CS, :], _NT,
                                   preferred_element_type=jnp.float32)

        S = {a: qk(items[a]) for a in range(AHEAD)}
        m = {}
        l = {}
        acc = {}
        for n, (h, j) in enumerate(items):
            if n + AHEAD < len(items):
                S[n + AHEAD] = qk(items[n + AHEAD])
            s = S.pop(n)
            mc = jnp.max(s, axis=-1, keepdims=True)
            m_new = mc if j == 0 else jnp.maximum(m[h], mc)
            p = jnp.exp2((s - m_new) * c_exp).astype(jnp.bfloat16)
            pv = jnp.dot(p, v_ref[h, j * CS:(j + 1) * CS, :],
                         preferred_element_type=jnp.float32)
            pf = p.astype(jnp.float32)
            ls = pf[:, :128]
            for t in range(1, CS // 128):
                ls = ls + pf[:, t * 128:(t + 1) * 128]
            if j == 0:
                l[h] = ls
                acc[h] = pv
            else:
                alpha = jnp.exp2((m[h] - m_new) * c_exp)
                l[h] = l[h] * alpha + ls
                acc[h] = acc[h] * alpha + pv
            m[h] = m_new
            if j == NC - 1:
                lsum = jnp.sum(l[h], axis=-1, keepdims=True)
                o_ref[h] = (acc[h] * pl.reciprocal(lsum, approx=False)).astype(o_ref.dtype)

    out = pl.pallas_call(
        kernel,
        grid=(G // hpb,),
        in_specs=[
            pl.BlockSpec((hpb, M, D), lambda i: (i, 0, 0)),
            pl.BlockSpec((hpb, Sk, D), lambda i: (i, 0, 0)),
            pl.BlockSpec((hpb, Sk, D), lambda i: (i, 0, 0)),
        ],
        out_specs=pl.BlockSpec((hpb, M, D), lambda i: (i, 0, 0)),
        out_shape=jax.ShapeDtypeStruct((G, M, D), q.dtype),
        compiler_params=pltpu.CompilerParams(
            dimension_semantics=("parallel",),
            vmem_limit_bytes=100 * 1024 * 1024),
    )(qr, kr, vr)
    return out.reshape(B, Hq, Sq, D)
```

```python
import math

import jax
import jax.numpy as jnp
from jax import lax
import jax.experimental.pallas as pl
import jax.experimental.pallas.tpu as pltpu

_NT = (((1,), (1,)), ((), ()))


@jax.jit
def pallas_standalone__gqa_softmax__near_ridge_kernel(
    q: jax.Array,
    k: jax.Array,
    v: jax.Array,
):
    B, Hq, Sq, D = q.shape
    Hkv, Sk = k.shape[1], k.shape[2]
    rep = Hq // Hkv
    M = rep * Sq
    G = B * Hkv
    NB = 8
    NO = 4
    N1 = 10
    N2 = (G - N1) // 2
    assert N1 + 2 * N2 == G and G >= NB
    qr = q.reshape(G, M, D)
    kr = k.reshape(G, Sk, D)
    vr = v.reshape(G, Sk, D)
    c_exp = (D ** -0.5) * math.log2(math.e)

    def kernel(q_hbm, k_hbm, v_hbm, o_hbm, qb, kb, vb, ob, sq, sk, sv, so):
        def in_copies(h):
            s = h & (NB - 1)
            return (pltpu.make_async_copy(q_hbm.at[h], qb.at[s], sq.at[s]),
                    pltpu.make_async_copy(k_hbm.at[h], kb.at[s], sk.at[s]),
                    pltpu.make_async_copy(v_hbm.at[h], vb.at[s], sv.at[s]))

        def o_copy(h):
            s = h & (NO - 1)
            return pltpu.make_async_copy(ob.at[s], o_hbm.at[h], so.at[s])

        def compute(h0, n, CS, ahead):
            NC = Sk // CS
            items = [(i, j) for j in range(NC) for i in range(n)]
            slot = [(h0 + i) & (NB - 1) for i in range(n)]
            oslot = [(h0 + i) & (NO - 1) for i in range(n)]

            def qk(it):
                i, j = it
                return lax.dot_general(qb[slot[i]], kb[slot[i], j * CS:(j + 1) * CS, :],
                                       _NT, preferred_element_type=jnp.float32)

            S = {a: qk(items[a]) for a in range(ahead)}
            m = {}
            l = {}
            acc = {}
            for t, (i, j) in enumerate(items):
                if t + ahead < len(items):
                    S[t + ahead] = qk(items[t + ahead])
                s = S.pop(t)
                mc = jnp.max(s, axis=-1, keepdims=True)
                m_new = mc if j == 0 else jnp.maximum(m[i], mc)
                p = jnp.exp2((s - m_new) * c_exp).astype(jnp.bfloat16)
                pv = jnp.dot(p, vb[slot[i], j * CS:(j + 1) * CS, :],
                             preferred_element_type=jnp.float32)
                pf = p.astype(jnp.float32)
                ls = pf[:, :128]
                for c in range(1, CS // 128):
                    ls = ls + pf[:, c * 128:(c + 1) * 128]
                if j == 0:
                    l[i] = ls
                    acc[i] = pv
                else:
                    alpha = jnp.exp2((m[i] - m_new) * c_exp)
                    l[i] = l[i] * alpha + ls
                    acc[i] = acc[i] * alpha + pv
                m[i] = m_new
                if j == NC - 1:
                    lsum = jnp.sum(l[i], axis=-1, keepdims=True)
                    ob[oslot[i]] = (acc[i] * pl.reciprocal(lsum, approx=False)
                                    ).astype(ob.dtype)

        def region(h0, n, CS, ahead):
            for i in range(n):
                @pl.when(h0 + i >= NO)
                def _():
                    o_copy(h0 + i - NO).wait()
            for i in range(n):
                for c in in_copies(h0 + i):
                    c.wait()
            compute(h0, n, CS, ahead)
            for i in range(n):
                o_copy(h0 + i).start()
            for i in range(n):
                @pl.when(h0 + i + NB < G)
                def _():
                    for c in in_copies(h0 + i + NB):
                        c.start()

        for h in range(NB):
            for c in in_copies(h):
                c.start()

        def body1(t, carry):
            region(t, 1, 512, 1)
            return carry
        lax.fori_loop(0, N1, body1, 0)

        def body2(t, carry):
            region(N1 + 2 * t, 2, 256, 2)
            return carry
        lax.fori_loop(0, N2, body2, 0)

        for h in range(G - NO, G):
            o_copy(h).wait()

    out = pl.pallas_call(
        kernel,
        in_specs=[pl.BlockSpec(memory_space=pl.ANY)] * 3,
        out_specs=pl.BlockSpec(memory_space=pl.ANY),
        out_shape=jax.ShapeDtypeStruct((G, M, D), q.dtype),
        scratch_shapes=[
            pltpu.VMEM((NB, M, D), q.dtype),
            pltpu.VMEM((NB, Sk, D), k.dtype),
            pltpu.VMEM((NB, Sk, D), v.dtype),
            pltpu.VMEM((NO, M, D), q.dtype),
            pltpu.SemaphoreType.DMA((NB,)),
            pltpu.SemaphoreType.DMA((NB,)),
            pltpu.SemaphoreType.DMA((NB,)),
            pltpu.SemaphoreType.DMA((NO,)),
        ],
        compiler_params=pltpu.CompilerParams(
            vmem_limit_bytes=100 * 1024 * 1024,
            disable_bounds_checks=True),
    )(qr, kr, vr)
    return out.reshape(B, Hq, Sq, D)
```

```python
import math

import jax
import jax.numpy as jnp
from jax import lax
import jax.experimental.pallas as pl
import jax.experimental.pallas.tpu as pltpu

_NT = (((1,), (1,)), ((), ()))


@jax.jit
def pallas_standalone__gqa_softmax__near_ridge_kernel(
    q: jax.Array,
    k: jax.Array,
    v: jax.Array,
):
    B, Hq, Sq, D = q.shape
    Hkv, Sk = k.shape[1], k.shape[2]
    rep = Hq // Hkv
    M = rep * Sq
    G = B * Hkv
    CS = 256
    AHEAD = 2
    NC = Sk // CS
    NB = 8
    N1 = 6
    N2 = (G - N1) // 2
    assert N1 + 2 * N2 == G and G >= NB and NC * CS == Sk
    TF = 0
    while N1 + 2 * (TF + 1) + NB < G + 2 and TF < N2 - 1:
        TF += 1
    HF = N1 + 2 * (TF + 1)
    NL = G - HF
    qr = q.reshape(G, M, D)
    kr = k.reshape(G, Sk, D)
    vr = v.reshape(G, Sk, D)
    c_exp = (D ** -0.5) * math.log2(math.e)

    def kernel(q_hbm, k_hbm, v_hbm, o_hbm, qb, kb, vb, ob, sq, sk, sv, sf, so):
        def in_copies(h):
            s = h & (NB - 1)
            return (pltpu.make_async_copy(q_hbm.at[h], qb.at[s], sq.at[s]),
                    pltpu.make_async_copy(k_hbm.at[h], kb.at[s], sk.at[s]),
                    pltpu.make_async_copy(v_hbm.at[h], vb.at[s], sv.at[s]))

        def flush_copy():
            return pltpu.make_async_copy(ob.at[pl.ds(0, HF)],
                                         o_hbm.at[pl.ds(0, HF)], sf.at[0])

        def o_copy(h):
            return pltpu.make_async_copy(ob.at[h], o_hbm.at[h], so.at[h - HF])

        def compute(h0, n):
            items = [(i, j) for j in range(NC) for i in range(n)]
            slot = [(h0 + i) & (NB - 1) for i in range(n)]

            def qk(it):
                i, j = it
                return lax.dot_general(qb[slot[i]], kb[slot[i], j * CS:(j + 1) * CS, :],
                                       _NT, preferred_element_type=jnp.float32)

            S = {a: qk(items[a]) for a in range(AHEAD)}
            m = {}
            l = {}
            acc = {}
            for t, (i, j) in enumerate(items):
                if t + AHEAD < len(items):
                    S[t + AHEAD] = qk(items[t + AHEAD])
                s = S.pop(t)
                mc = jnp.max(s, axis=-1, keepdims=True)
                m_new = mc if j == 0 else jnp.maximum(m[i], mc)
                p = jnp.exp2((s - m_new) * c_exp).astype(jnp.bfloat16)
                pv = jnp.dot(p, vb[slot[i], j * CS:(j + 1) * CS, :],
                             preferred_element_type=jnp.float32)
                pf = p.astype(jnp.float32)
                ls = pf[:, :128]
                for c in range(1, CS // 128):
                    ls = ls + pf[:, c * 128:(c + 1) * 128]
                if j == 0:
                    l[i] = ls
                    acc[i] = pv
                else:
                    alpha = jnp.exp2((m[i] - m_new) * c_exp)
                    l[i] = l[i] * alpha + ls
                    acc[i] = acc[i] * alpha + pv
                m[i] = m_new
                if j == NC - 1:
                    lsum = jnp.sum(l[i], axis=-1, keepdims=True)
                    ob[h0 + i] = (acc[i] * pl.reciprocal(lsum, approx=False)
                                  ).astype(ob.dtype)

        def region(h0, n):
            for i in range(n):
                for c in in_copies(h0 + i):
                    c.wait()
            compute(h0, n)
            for i in range(n):
                @pl.when(h0 + i + NB < G)
                def _():
                    for c in in_copies(h0 + i + NB):
                        c.start()

        for h in range(NB):
            for c in in_copies(h):
                c.start()

        def body1(t, carry):
            region(t, 1)
            return carry
        lax.fori_loop(0, N1, body1, 0)

        def body2(t, carry):
            h0 = N1 + 2 * t
            region(h0, 2)

            @pl.when(t == TF)
            def _():
                flush_copy().start()

            if NL > 0:
                @pl.when(t > TF)
                def _():
                    for i in range(2):
                        o_copy(h0 + i).start()
            return carry
        lax.fori_loop(0, N2, body2, 0)

        flush_copy().wait()
        for h in range(HF, G):
            o_copy(h).wait()

    out = pl.pallas_call(
        kernel,
        in_specs=[pl.BlockSpec(memory_space=pl.ANY)] * 3,
        out_specs=pl.BlockSpec(memory_space=pl.ANY),
        out_shape=jax.ShapeDtypeStruct((G, M, D), q.dtype),
        scratch_shapes=[
            pltpu.VMEM((NB, M, D), q.dtype),
            pltpu.VMEM((NB, Sk, D), k.dtype),
            pltpu.VMEM((NB, Sk, D), v.dtype),
            pltpu.VMEM((G, M, D), q.dtype),
            pltpu.SemaphoreType.DMA((NB,)),
            pltpu.SemaphoreType.DMA((NB,)),
            pltpu.SemaphoreType.DMA((NB,)),
            pltpu.SemaphoreType.DMA((1,)),
            pltpu.SemaphoreType.DMA((max(NL, 1),)),
        ],
        compiler_params=pltpu.CompilerParams(
            vmem_limit_bytes=100 * 1024 * 1024,
            disable_bounds_checks=True),
    )(qr, kr, vr)
    return out.reshape(B, Hq, Sq, D)
```

```python
import math

import jax
import jax.numpy as jnp
from jax import lax
import jax.experimental.pallas as pl
import jax.experimental.pallas.tpu as pltpu

_NT = (((1,), (1,)), ((), ()))


@jax.jit
def pallas_standalone__gqa_softmax__near_ridge_kernel(
    q: jax.Array,
    k: jax.Array,
    v: jax.Array,
):
    B, Hq, Sq, D = q.shape
    Hkv, Sk = k.shape[1], k.shape[2]
    rep = Hq // Hkv
    M = rep * Sq
    G = B * Hkv
    CS = 256
    AHEAD = 2
    NC = Sk // CS
    JS = 3
    KS = JS * CS
    NB = 8
    N1 = 6
    N2 = (G - N1) // 2
    assert N1 + 2 * N2 == G and G > NB and NC * CS == Sk and JS < NC
    TF = 0
    while N1 + 2 * (TF + 1) + NB < G + 2 and TF < N2 - 1:
        TF += 1
    HF = N1 + 2 * (TF + 1)
    NL = G - HF
    qr = q.reshape(G, M, D)
    kr = k.reshape(G, Sk, D)
    vr = v.reshape(G, Sk, D)
    c_exp = (D ** -0.5) * math.log2(math.e)

    def kernel(q_hbm, k_hbm, v_hbm, o_hbm, qb, kb, vb, ob, sq, sk, sv, s0, sf, so):
        def in_copies(h):
            s = h & (NB - 1)
            return (pltpu.make_async_copy(q_hbm.at[h], qb.at[s], sq.at[s]),
                    pltpu.make_async_copy(k_hbm.at[h], kb.at[s], sk.at[s]),
                    pltpu.make_async_copy(v_hbm.at[h], vb.at[s], sv.at[s]))

        def first_copies(part):
            lo, n = (0, KS) if part == 0 else (KS, Sk - KS)
            cs = [pltpu.make_async_copy(k_hbm.at[0, pl.ds(lo, n)],
                                        kb.at[0, pl.ds(lo, n)], s0.at[2 * part]),
                  pltpu.make_async_copy(v_hbm.at[0, pl.ds(lo, n)],
                                        vb.at[0, pl.ds(lo, n)], s0.at[2 * part + 1])]
            if part == 0:
                cs = [pltpu.make_async_copy(q_hbm.at[0], qb.at[0], sq.at[0])] + cs
            return cs

        def flush_copy():
            return pltpu.make_async_copy(ob.at[pl.ds(0, HF)],
                                         o_hbm.at[pl.ds(0, HF)], sf.at[0])

        def o_copy(h):
            return pltpu.make_async_copy(ob.at[h], o_hbm.at[h], so.at[h - HF])

        def compute(h0, n, j_lo=0, j_hi=NC, state=None, out_pred=None):
            items = [(i, j) for j in range(j_lo, j_hi) for i in range(n)]
            slot = [(h0 + i) & (NB - 1) for i in range(n)]

            def qk(it):
                i, j = it
                return lax.dot_general(qb[slot[i]], kb[slot[i], j * CS:(j + 1) * CS, :],
                                       _NT, preferred_element_type=jnp.float32)

            S = {a: qk(items[a]) for a in range(min(AHEAD, len(items)))}
            m, l, acc = state if state is not None else ({}, {}, {})
            for t, (i, j) in enumerate(items):
                if t + AHEAD < len(items):
                    S[t + AHEAD] = qk(items[t + AHEAD])
                s = S.pop(t)
                mc = jnp.max(s, axis=-1, keepdims=True)
                m_new = mc if j == 0 else jnp.maximum(m[i], mc)
                p = jnp.exp2((s - m_new) * c_exp).astype(jnp.bfloat16)
                pv = jnp.dot(p, vb[slot[i], j * CS:(j + 1) * CS, :],
                             preferred_element_type=jnp.float32)
                pf = p.astype(jnp.float32)
                ls = pf[:, :128]
                for c in range(1, CS // 128):
                    ls = ls + pf[:, c * 128:(c + 1) * 128]
                if j == 0:
                    l[i] = ls
                    acc[i] = pv
                else:
                    alpha = jnp.exp2((m[i] - m_new) * c_exp)
                    l[i] = l[i] * alpha + ls
                    acc[i] = acc[i] * alpha + pv
                m[i] = m_new
                if j == NC - 1:
                    lsum = jnp.sum(l[i], axis=-1, keepdims=True)
                    ob[h0 + i] = (acc[i] * pl.reciprocal(lsum, approx=False)
                                  ).astype(ob.dtype)
                    if out_pred is not None:
                        @pl.when(out_pred)
                        def _():
                            o_copy(h0 + i).start()
            return m, l, acc

        def region(h0, n, out_pred=None):
            for i in range(n):
                for c in in_copies(h0 + i):
                    c.wait()
            compute(h0, n, out_pred=out_pred)
            for i in range(n):
                @pl.when(h0 + i + NB < G)
                def _():
                    for c in in_copies(h0 + i + NB):
                        c.start()

        for c in first_copies(0) + first_copies(1):
            c.start()
        for h in range(1, NB):
            for c in in_copies(h):
                c.start()

        for c in first_copies(0):
            c.wait()
        state = compute(0, 1, 0, JS)
        for c in first_copies(1):
            c.wait()
        compute(0, 1, JS, NC, state)
        for c in in_copies(NB):
            c.start()

        def body1(t, carry):
            region(t, 1)
            return carry
        lax.fori_loop(1, N1, body1, 0)

        def body2(t, carry):
            region(N1 + 2 * t, 2, out_pred=(t > TF) if NL > 0 else None)

            @pl.when(t == TF)
            def _():
                flush_copy().start()
            return carry
        lax.fori_loop(0, N2, body2, 0)

        flush_copy().wait()
        for h in range(HF, G):
            o_copy(h).wait()

    out = pl.pallas_call(
        kernel,
        in_specs=[pl.BlockSpec(memory_space=pl.ANY)] * 3,
        out_specs=pl.BlockSpec(memory_space=pl.ANY),
        out_shape=jax.ShapeDtypeStruct((G, M, D), q.dtype),
        scratch_shapes=[
            pltpu.VMEM((NB, M, D), q.dtype),
            pltpu.VMEM((NB, Sk, D), k.dtype),
            pltpu.VMEM((NB, Sk, D), v.dtype),
            pltpu.VMEM((G, M, D), q.dtype),
            pltpu.SemaphoreType.DMA((NB,)),
            pltpu.SemaphoreType.DMA((NB,)),
            pltpu.SemaphoreType.DMA((NB,)),
            pltpu.SemaphoreType.DMA((4,)),
            pltpu.SemaphoreType.DMA((1,)),
            pltpu.SemaphoreType.DMA((max(NL, 1),)),
        ],
        compiler_params=pltpu.CompilerParams(
            vmem_limit_bytes=100 * 1024 * 1024,
            disable_bounds_checks=True),
    )(qr, kr, vr)
    return out.reshape(B, Hq, Sq, D)
```
